```python
import os as _os
_os.environ.setdefault("JAX_PLATFORMS", "cpu")
import jax
import jax.numpy as jnp

def _softmax(x, axis=-1):
    return jax.nn.softmax(x, axis=axis)
def _gelu(x):
    return jax.nn.gelu(x, approximate=True)
def _silu(x):
    return jax.nn.silu(x)
def _sigmoid(x):
    return jax.nn.sigmoid(x)
def _layernorm(x, axis=-1, eps=1e-5):
    m = jnp.mean(x, axis=axis, keepdims=True)
    v = jnp.var(x, axis=axis, keepdims=True)
    return (x - m) / jnp.sqrt(v + eps)
def _scatter_add(tgt, idx, src, axis=0):
    return tgt.at[idx].add(src)
def _segment_sum(src, seg, n):
    return jax.ops.segment_sum(src, seg, n)
class _Rng:
    def __init__(self, key):
        self._k = key
    def _next(self):
        self._k, sub = jax.random.split(self._k)
        return sub
    def normal(self, shape):
        return jax.random.normal(self._next(), shape, dtype=jnp.bfloat16)
    def randint(self, lo, hi, shape):
        return jax.random.randint(self._next(), shape, lo, hi, dtype=jnp.int32)
    def uniform(self, shape, lo=0.0, hi=1.0):
        return jax.random.uniform(self._next(), shape, jnp.bfloat16, lo, hi)
    def permutation(self, n):
        return jax.random.permutation(self._next(), n)


kernel_name = 'gated_mix__softmax_full_mha__dense_activation_relu__prompt'

def setup_inputs():
    _rng = _Rng(jax.random.key(int.from_bytes(__import__("os").urandom(4), "little")))
    _w = (lambda a: (lambda t: t.astype(jnp.bfloat16) if jnp.issubdtype(t.dtype, jnp.floating) else t)(jnp.asarray(a)))
    def _A_setup():
        B, S, D = 1, 2048, 640
        return {
            "x": _w((lambda *s: _rng.normal(s) * 0.05)(B, S, D)),
            "wqkv": _w((lambda *s: _rng.normal(s) * 0.8)(D, 3 * D)),
            "wo": _w((lambda *s: _rng.normal(s) * 0.05)(D, D)),
        }
    _A_in = _A_setup()

    def _B_setup():
        B, S, D, Dff = 1, 2048, 640, 1536
        return {
            "x": _w((lambda *s: _rng.normal(s) * 0.05)(B, S, D)),
            "w1": _w((lambda *s: _rng.normal(s) * 0.05)(D, Dff)),
            "w2": _w((lambda *s: _rng.normal(s) * 0.05)(Dff, D)),
        }
    _B_in = _B_setup()

    return {
        "A_x": _A_in["x"],
        "A_wqkv": _A_in["wqkv"],
        "A_wo": _A_in["wo"],
        "B_x": _B_in["x"],
        "B_w1": _B_in["w1"],
        "B_w2": _B_in["w2"],
        "gate_w": _w((lambda *s: _rng.normal(s) * 0.05)(640) * 16.0),
    }

def reference(A_x, A_wqkv, A_wo, B_x, B_w1, B_w2, gate_w):
    def _A_ref(x, wqkv, wo):
        B, S, D = x.shape
        H = 32; Dh = D // H
        qkv = (lambda x, *d: x.transpose(*d))((x @ wqkv).reshape(B, S, 3, H, Dh), 2, 0, 3, 1, 4)
        q, k, v = qkv[0], qkv[1], qkv[2]
        scale = Dh ** -0.5
        scores = jnp.einsum("bhqd,bhkd->bhqk", q, k) * scale
        p = _softmax(scores, axis=-1)
        o = jnp.einsum("bhqk,bhkd->bhqd", p, v)
        return (lambda x, *d: x.transpose(*d))(o, 0, 2, 1, 3).reshape(B, S, D) @ wo

    def _B_ref(x, w1, w2):
        h = jnp.einsum("bsd,df->bsf", x, w1)
        zero = jnp.zeros_like(h)
        h = jnp.maximum(h, zero)
        return jnp.einsum("bsf,fd->bsd", h, w2)

    x = A_x
    g = _sigmoid((x * gate_w).sum(-1, keepdims=True))
    a = _A_ref(x, A_wqkv, A_wo)
    b = _B_ref(x, B_w1, B_w2)
    return g * a + (1 - g) * b
```

```python
import math

import jax
import jax.numpy as jnp
from jax import lax
from jax.experimental import pallas as pl
from jax.experimental.pallas import tpu as pltpu

S, D, H, DH, DFF = 2048, 640, 32, 20, 1536
TM = 512
BQ = 512
KC = 128
NQ, NC = S // BQ, S // KC
UNROLL = 8
LAG = 1
VR = 24
F32, BF16, U32 = jnp.float32, jnp.bfloat16, jnp.uint32
QSCALE = DH ** -0.5 * math.log2(math.e)
NN = (((1,), (0,)), ((), ()))
NT = (((1,), (1,)), ((), ()))
TN = (((0,), (0,)), ((), ()))


def _dot(a, b, dims=NN):
    return lax.dot_general(a, b, dims, preferred_element_type=F32)


def _kernel(x_hbm, wqkv_hbm, wo_hbm, w1_hbm, w2_hbm, gw_ref, o_hbm,
            x_v, wqkv_v, wo_v, w1_v, w2_v, wqvt, kp, qt, vw, oraw, s0, s1,
            out_v, sem_x, sem_w, sem_o):
    nchunk = S // TM
    x_cp = [pltpu.make_async_copy(x_hbm.at[pl.ds(i * TM, TM)],
                                  x_v.at[pl.ds(i * TM, TM)], sem_x.at[i])
            for i in range(nchunk)]
    w_cp = [pltpu.make_async_copy(s, d, sem_w.at[i]) for i, (s, d) in enumerate(
        [(wqkv_hbm, wqkv_v), (w1_hbm, w1_v), (w2_hbm, w2_v), (wo_hbm, wo_v)])]
    w_cp[0].start()
    for c in x_cp:
        c.start()
    for c in w_cp[1:]:
        c.start()

    w_cp[0].wait()
    wqvt[0:D, :] = wqkv_v[:, 0:D].T
    wqvt[D:2 * D, :] = wqkv_v[:, 2 * D:3 * D].T

    def proj(i, carry):
        pltpu.make_async_copy(x_hbm.at[pl.ds(0, TM)], x_v.at[pl.ds(0, TM)],
                              sem_x.at[i]).wait()
        r0 = pl.multiple_of(i * TM, TM)
        xc = x_v[pl.ds(r0, TM), :]
        k = pltpu.bitcast(_dot(xc, wqkv_v[:, D:2 * D]).astype(BF16), U32)
        rows = pl.ds(pl.multiple_of(i * (TM // 2), TM // 2), TM // 2)
        hi = lax.broadcasted_iota(jnp.int32, (TM // 2, 128), 1) >= 64
        for j in range(5):
            kp[j, rows, :] = k[:, j * 128:(j + 1) * 128]
        for j in range(4):
            kp[5 + j, rows, :] = jnp.where(hi, k[:, j * 128:(j + 1) * 128],
                                           k[:, (j + 1) * 128:(j + 2) * 128])
        cols = pl.ds(r0, TM)
        q = _dot(wqvt[0:D, :], xc, NT) * QSCALE
        row32 = lax.broadcasted_iota(jnp.int32, (32, TM), 0)
        zero = jnp.zeros((8, TM), U32)
        for h in range(H):
            ws, off = divmod(h * DH, 16)
            win = q[ws * 16:ws * 16 + 32, :]
            win = jnp.where((row32 >= off) & (row32 < off + DH), win, 0.0)
            win = pltpu.bitcast(win.astype(BF16), U32)
            for t in range(8):
                val = win[0:8] if t == ws % 8 else (
                    win[8:16] if t == (ws + 1) % 8 else zero)
                qt[h, t * 8:(t + 1) * 8, cols] = val
        v = _dot(wqvt[D:2 * D, :], xc, NT).astype(BF16).astype(F32)
        row24 = lax.broadcasted_iota(jnp.int32, (VR, TM), 0)
        for h in range(H):
            ws, off = divmod(h * DH, 8)
            win = v[ws * 8:ws * 8 + VR, :]
            vw[h, :, cols] = jnp.where(row24 == (DH if off == 0 else 0), 1.0, win)
        return carry

    lax.fori_loop(0, nchunk, proj, 0)

    sb = (s0, s1)

    def qk(u, par, c, mx):
        h, qb = u // NQ, u % NQ
        ws = (h * DH) // 16
        if isinstance(u, int):
            ki = 5 + ws // 8 if ws % 8 == 7 else ws // 8
            cols = pl.ds(qb * BQ, BQ)
        else:
            ki = jnp.where(ws % 8 == 7, 5, 0) + ws // 8
            cols = pl.ds(pl.multiple_of(qb * BQ, BQ), BQ)
        q = pltpu.bitcast(qt[h, :, cols], BF16)
        k = pltpu.bitcast(kp[ki, c * KC // 2:(c + 1) * KC // 2, :], BF16)
        s = _dot(k, q)
        sb[par][c * KC:(c + 1) * KC, :] = s
        mc = jnp.max(s.reshape(KC // 8, 8, BQ), axis=0)
        return mc if c == 0 else jnp.maximum(mx, mc)

    def pv(u, par, c, m, acc):
        h, qb = u // NQ, u % NQ
        sl = slice(c * KC, (c + 1) * KC)
        p = jnp.exp2(sb[par][sl, :] - m).astype(BF16)
        o = _dot(vw[h, :, sl], p)
        acc = o if c == 0 else acc + o
        if c == NC - 1:
            oraw[qb, h] = acc
        return acc

    def step(u, par, st, do_qk=True, do_pv2=True, do_pv1=True):
        m2, m1, acc = st
        mx = None
        for c in range(NC):
            if do_qk:
                mx = qk(u, par, c, mx)
            if c < LAG:
                if do_pv2:
                    acc = pv(u - 2, par, NC - LAG + c, m2, acc)
            elif do_pv1:
                acc = pv(u - 1, 1 - par, c - LAG, m1, acc)
        m0 = jnp.max(mx, axis=0, keepdims=True) if do_qk else m1
        return m1, m0, acc

    n = H * NQ
    z = jnp.zeros((1, BQ), F32)
    st = (z, z, jnp.zeros((VR, BQ), F32))
    st = step(0, 0, st, True, False, False)
    st = step(1, 1, st, True, False, True)

    def body(i, st):
        for t in range(UNROLL):
            st = step(2 + i * UNROLL + t, t % 2, st)
        return st

    nit = (n - 2) // UNROLL
    st = lax.fori_loop(0, nit, body, st)
    for u in range(2 + nit * UNROLL, n):
        st = step(u, u % 2, st)
    st = step(n, 0, st, False, True, True)
    st = step(n + 1, 1, st, False, True, False)

    for c in w_cp[1:]:
        c.wait()

    def out_copy(i):
        r = pl.ds(pl.multiple_of(i * TM, TM), TM)
        return pltpu.make_async_copy(out_v.at[r], o_hbm.at[r], sem_o.at[i])

    def tail(i, carry):
        rows = pl.ds(pl.multiple_of(i * TM, TM), TM)
        xc = x_v[rows, :]
        hid = jnp.maximum(_dot(xc, w1_v[...]), 0.0).astype(BF16)
        b = _dot(hid, w2_v[...])
        low = lax.broadcasted_iota(jnp.int32, (8, TM), 0) < 4
        parts = []
        for hp in range(H // 2):
            e = oraw[i, 2 * hp]
            o = oraw[i, 2 * hp + 1]
            e = e * (1.0 / e[DH:DH + 1, :])
            o = o * (1.0 / o[0:1, :])
            parts += [e[0:16], jnp.where(low, e[16:24], o[0:8]), o[8:24]]
        ot = jnp.concatenate(parts, axis=0).astype(BF16)
        a = _dot(ot, wo_v[...], TN)
        gl = jnp.sum(xc.astype(F32) * gw_ref[...].astype(F32), axis=-1, keepdims=True)
        g = 1.0 / (1.0 + jnp.exp(-gl))
        out_v[rows, :] = (g * a + (1.0 - g) * b).astype(BF16)
        out_copy(i).start()
        return carry

    lax.fori_loop(0, nchunk, tail, 0)
    for i in range(nchunk):
        out_copy(i).wait()


@jax.jit
def pallas_gated_mix__softmax_full_mha__dense_activation_relu__prompt_kernel(
    A_x: jax.Array,
    A_wqkv: jax.Array,
    A_wo: jax.Array,
    B_x: jax.Array,
    B_w1: jax.Array,
    B_w2: jax.Array,
    gate_w: jax.Array,
):
    del B_x
    assert TM == BQ
    any_spec = pl.BlockSpec(memory_space=pl.ANY)
    out = pl.pallas_call(
        _kernel,
        out_shape=jax.ShapeDtypeStruct((S, D), BF16),
        in_specs=[any_spec] * 5 + [pl.BlockSpec(memory_space=pltpu.VMEM)],
        out_specs=any_spec,
        scratch_shapes=[
            pltpu.VMEM((S, D), BF16),
            pltpu.VMEM((D, 3 * D), BF16),
            pltpu.VMEM((D, D), BF16),
            pltpu.VMEM((D, DFF), BF16),
            pltpu.VMEM((DFF, D), BF16),
            pltpu.VMEM((2 * D, D), BF16),
            pltpu.VMEM((9, S // 2, 128), U32),
            pltpu.VMEM((H, 64, S), U32),
            pltpu.VMEM((H, VR, S), F32),
            pltpu.VMEM((NQ, H, VR, BQ), F32),
            pltpu.VMEM((S, BQ), F32),
            pltpu.VMEM((S, BQ), F32),
            pltpu.VMEM((S, D), BF16),
            pltpu.SemaphoreType.DMA((S // TM,)),
            pltpu.SemaphoreType.DMA((4,)),
            pltpu.SemaphoreType.DMA((S // TM,)),
        ],
        compiler_params=pltpu.CompilerParams(vmem_limit_bytes=100 * 2 ** 20),
        name="gated_mix_mha_ffn",
    )(A_x.reshape(S, D), A_wqkv, A_wo, B_w1, B_w2, gate_w.reshape(1, D))
    return out.reshape(1, S, D)
```

```python
import math

import jax
import jax.numpy as jnp
from jax import lax
from jax.experimental import pallas as pl
from jax.experimental.pallas import tpu as pltpu

S, D, H, DH, DFF = 2048, 640, 32, 20, 1536
TM = 512
KC = 128
NQ, NC = S // TM, S // KC
HEADS = 2
VR = 24
TL = 128
ZH = 20
FILL = 128
F32, BF16, U32 = jnp.float32, jnp.bfloat16, jnp.uint32
QSCALE = DH ** -0.5 * math.log2(math.e)
NN = (((1,), (0,)), ((), ()))
NT = (((1,), (1,)), ((), ()))
TN = (((0,), (0,)), ((), ()))


def _dot(a, b, dims=NN):
    return lax.dot_general(a, b, dims, preferred_element_type=F32)


def _ds(start, size):
    return pl.ds(start if isinstance(start, int) else pl.multiple_of(start, size), size)


def _kernel(x_hbm, wqkv_hbm, wo_hbm, w1_hbm, w2_hbm, gw_hbm, o_hbm,
            x_v, wqkv_v, wo_v, w1_v, w2_v, gw_v, wqvt, kp, qt, vw, oraw, s0, s1,
            hid0, out_v, sem_x, sem_w, sem_o):
    x_cp = [pltpu.make_async_copy(x_hbm.at[pl.ds(i * TM, TM)], x_v.at[pl.ds(i * TM, TM)],
                                  sem_x.at[i]) for i in range(NQ)]
    wq_cp, wk_cp, wv_cp = [
        pltpu.make_async_copy(wqkv_hbm.at[:, pl.ds(j * D, D)], wqkv_v.at[j], sem_w.at[j])
        for j in range(3)]
    w_cp = [pltpu.make_async_copy(s, d, sem_w.at[3 + i]) for i, (s, d) in enumerate(
        [(w1_hbm, w1_v), (w2_hbm, w2_v), (wo_hbm, wo_v), (gw_hbm, gw_v)])]

    def k_proj(i):
        xc = x_v[i * TM:(i + 1) * TM, :]
        k = jnp.concatenate([
            _dot(xc, wqkv_v[1, :, :512]),
            jnp.concatenate([_dot(xc[r:r + TM // 4], wqkv_v[1, :, 512:])
                             for r in range(0, TM, TM // 4)], axis=0)], axis=1)
        k = pltpu.bitcast(k.astype(BF16), U32)
        tiles = [k[:, j * 128:(j + 1) * 128] for j in range(5)]
        rows = slice(i * TM // 2, (i + 1) * TM // 2)
        hi = lax.broadcasted_iota(jnp.int32, (TM // 2, 128), 1) >= 64
        for j in range(5):
            kp[j, rows, :] = tiles[j]
        for j in range(4):
            kp[5 + j, rows, :] = jnp.where(hi, tiles[j], tiles[j + 1])

    def clear_q(h, carry=None):
        qt[h] = jnp.zeros(qt.shape[1:], U32)
        return carry

    wk_cp.start()
    x_cp[0].start()
    lax.fori_loop(0, ZH, clear_q, 0)
    s0[S - KC:, :] = jnp.zeros((KC, TM), F32)
    s1[...] = jnp.zeros((S, TM), F32)
    wk_cp.wait()
    starts = ([x_cp[1], x_cp[2]], [x_cp[3], wq_cp], [wv_cp], w_cp)
    for i in range(NQ):
        x_cp[i].wait()
        if i == 2:
            wq_cp.wait()
        if i == 3:
            wv_cp.wait()
        for c in starts[i]:
            c.start()
        k_proj(i)
        for h in range(ZH + (H - ZH) * i // NQ, ZH + (H - ZH) * (i + 1) // NQ):
            clear_q(h)
        if i == 2:
            wqvt[0] = wqkv_v[0].T
        if i == 3:
            wqvt[1] = wqkv_v[2].T

    def proj(i, carry):
        cols = _ds(i * TM, TM)
        xc = x_v[cols, :]
        q = _dot(wqvt[0], xc, NT) * QSCALE
        row = lax.broadcasted_iota(jnp.int32, (32, TM), 0)
        for h in range(H):
            ws, off = divmod(h * DH, 16)
            win = jnp.where((row >= off) & (row < off + DH), q[ws * 16:ws * 16 + 32], 0.0)
            win = pltpu.bitcast(win.astype(BF16), U32)
            for t in range(2):
                p = (ws + t) % 8
                qt[h, p * 8:(p + 1) * 8, cols] = win[t * 8:(t + 1) * 8]
        v = _dot(wqvt[1], xc, NT).astype(BF16).astype(F32)
        row = lax.broadcasted_iota(jnp.int32, (VR, TM), 0)
        for h in range(H):
            ws, off = divmod(h * DH, 8)
            vw[h, :, cols] = jnp.where(row == (0 if off else DH), 1.0, v[ws * 8:ws * 8 + VR])
        return carry

    lax.fori_loop(0, NQ, proj, 0)
    for c in w_cp:
        c.wait()

    sb = (s0, s1)

    def qk(h, qb, c, mx):
        ws = (h * DH) >> 4
        slab = jnp.where((ws & 7) == 7, 5, 0) + (ws >> 3)
        q = pltpu.bitcast(qt[h, :, qb * TM:(qb + 1) * TM], BF16)
        k = pltpu.bitcast(kp[slab, c * KC // 2:(c + 1) * KC // 2, :], BF16)
        s = _dot(k, q)
        sb[qb % 2][c * KC:(c + 1) * KC, :] = s
        mc = jnp.max(s.reshape(KC // 8, 8, TM), axis=0)
        return mc if c == 0 else jnp.maximum(mx, mc)

    def pv(h, qb, c, m, acc):
        keys = slice(c * KC, (c + 1) * KC)
        p = jnp.exp2(sb[qb % 2][keys, :] - m).astype(BF16)
        o = _dot(vw[h, :, keys], p)
        acc = o if c == 0 else acc + o
        if c == NC - 1:
            oraw[qb, h] = acc
        return acc

    def attend(i, state):
        def unit(t):
            h = i * HEADS + t // NQ
            return (jnp.maximum(h, 0) if t < 0 else h), t % NQ

        m2, m1, acc = state
        for t in range(HEADS * NQ):
            mx = None
            for c in range(NC):
                mx = qk(*unit(t), c, mx)
                if c == 0:
                    acc = pv(*unit(t - 2), NC - 1, m2, acc)
                else:
                    acc = pv(*unit(t - 1), c - 1, m1, acc)
            m2, m1 = m1, jnp.max(mx, axis=0, keepdims=True)
        return m2, m1, acc

    zero = jnp.zeros((1, TM), F32)
    m2, m1, acc = lax.fori_loop(0, H // HEADS, attend,
                                (zero, zero, jnp.zeros((VR, TM), F32)))
    acc = pv(H - 1, NQ - 2, NC - 1, m2, acc)
    for c in range(NC):
        rows = slice(c * KC, (c + 1) * KC)
        hid0[rows, :] = jnp.maximum(_dot(x_v[rows, :], w1_v[:, :FILL]), 0.0).astype(BF16)
        acc = pv(H - 1, NQ - 1, c, m1, acc)

    def out_copy(i):
        rows = _ds(i * TL, TL)
        return pltpu.make_async_copy(out_v.at[rows], o_hbm.at[rows], sem_o.at[i])

    def tail(i, carry):
        rows = _ds(i * TM, TM)
        xc = x_v[rows, :]
        hid = jnp.maximum(_dot(xc, w1_v[:, FILL:]), 0.0).astype(BF16)
        b = _dot(jnp.concatenate([hid0[rows, :], hid], axis=1), w2_v[...])
        low = lax.broadcasted_iota(jnp.int32, (8, TM), 0) < 4
        parts = []
        for hp in range(H // 2):
            e, o = oraw[i, 2 * hp], oraw[i, 2 * hp + 1]
            e = e * (1.0 / e[DH:DH + 1])
            o = o * (1.0 / o[0:1])
            parts += [e[0:16], jnp.where(low, e[16:24], o[0:8]), o[8:24]]
        a = _dot(jnp.concatenate(parts, axis=0).astype(BF16), wo_v[...], TN)
        gw = gw_v[...].reshape(1, D).astype(F32)
        g = 1.0 / (1.0 + jnp.exp(-jnp.sum(xc.astype(F32) * gw, axis=-1, keepdims=True)))
        out = (g * a + (1.0 - g) * b).astype(BF16)
        for j in range(TM // TL):
            out_v[_ds(i * TM + j * TL, TL), :] = out[j * TL:(j + 1) * TL]
            out_copy(i * (TM // TL) + j).start()
        return carry

    lax.fori_loop(0, NQ, tail, 0)
    for i in range(S // TL):
        out_copy(i).wait()


@jax.jit
def pallas_gated_mix__softmax_full_mha__dense_activation_relu__prompt_kernel(
    A_x: jax.Array,
    A_wqkv: jax.Array,
    A_wo: jax.Array,
    B_x: jax.Array,
    B_w1: jax.Array,
    B_w2: jax.Array,
    gate_w: jax.Array,
):
    del B_x
    hbm = pl.BlockSpec(memory_space=pl.ANY)
    out = pl.pallas_call(
        _kernel,
        out_shape=jax.ShapeDtypeStruct((S, D), BF16),
        in_specs=[hbm] * 6,
        out_specs=hbm,
        scratch_shapes=[
            pltpu.VMEM((S, D), BF16),
            pltpu.VMEM((3, D, D), BF16),
            pltpu.VMEM((D, D), BF16),
            pltpu.VMEM((D, DFF), BF16),
            pltpu.VMEM((DFF, D), BF16),
            pltpu.VMEM((D,), BF16),
            pltpu.VMEM((2, D, D), BF16),
            pltpu.VMEM((9, S // 2, 128), U32),
            pltpu.VMEM((H, 64, S), U32),
            pltpu.VMEM((H, VR, S), F32),
            pltpu.VMEM((NQ, H, VR, TM), F32),
            pltpu.VMEM((S, TM), F32),
            pltpu.VMEM((S, TM), F32),
            pltpu.VMEM((S, FILL), BF16),
            pltpu.VMEM((S, D), BF16),
            pltpu.SemaphoreType.DMA((NQ,)),
            pltpu.SemaphoreType.DMA((7,)),
            pltpu.SemaphoreType.DMA((S // TL,)),
        ],
        compiler_params=pltpu.CompilerParams(vmem_limit_bytes=100 * 2 ** 20),
        name="gated_mix_mha_ffn",
    )(A_x.reshape(S, D), A_wqkv, A_wo, B_w1, B_w2, gate_w)
    return out.reshape(1, S, D)
```
